```python
import os as _os
_os.environ.setdefault("JAX_PLATFORMS", "cpu")
import jax
import jax.numpy as jnp

def _softmax(x, axis=-1):
    return jax.nn.softmax(x, axis=axis)
def _gelu(x):
    return jax.nn.gelu(x, approximate=True)
def _silu(x):
    return jax.nn.silu(x)
def _sigmoid(x):
    return jax.nn.sigmoid(x)
def _layernorm(x, axis=-1, eps=1e-5):
    m = jnp.mean(x, axis=axis, keepdims=True)
    v = jnp.var(x, axis=axis, keepdims=True)
    return (x - m) / jnp.sqrt(v + eps)
def _scatter_add(tgt, idx, src, axis=0):
    return tgt.at[idx].add(src)
def _segment_sum(src, seg, n):
    return jax.ops.segment_sum(src, seg, n)
class _Rng:
    def __init__(self, key):
        self._k = key
    def _next(self):
        self._k, sub = jax.random.split(self._k)
        return sub
    def normal(self, shape):
        return jax.random.normal(self._next(), shape, dtype=jnp.bfloat16)
    def randint(self, lo, hi, shape):
        return jax.random.randint(self._next(), shape, lo, hi, dtype=jnp.int32)
    def uniform(self, shape, lo=0.0, hi=1.0):
        return jax.random.uniform(self._next(), shape, jnp.bfloat16, lo, hi)
    def permutation(self, n):
        return jax.random.permutation(self._next(), n)


kernel_name = 'standalone__sliding_local_fixed_window__prompt'

def setup_inputs():
    _rng = _Rng(jax.random.key(int.from_bytes(__import__("os").urandom(4), "little")))
    _w = (lambda a: (lambda t: t.astype(jnp.bfloat16) if jnp.issubdtype(t.dtype, jnp.floating) else t)(jnp.asarray(a)))
    B, H, S, D = 1, 32, 2048, 128
    return {
        "q": _w((lambda *s: _rng.normal(s) * 0.4)(B, H, S, D)),
        "k": _w((lambda *s: _rng.normal(s) * 0.4)(B, H, S, D)),
        "v": _w((lambda *s: _rng.normal(s) * 0.05)(B, H, S, D)),
    }

def reference(q, k, v):
    B, H, S, D = q.shape
    w = 32
    pos = jnp.arange(S)
    rel = pos[:, None] - pos[None, :]
    mask = (rel >= 0) & (rel < w)
    scores = jnp.einsum("bhqd,bhkd->bhqk", q, k) * (D ** -0.5)
    scores = jnp.where(mask[None, None], scores, (lambda x, dt: x.astype(dt))(jnp.array(-1e9), q.dtype))
    p = _softmax(scores, axis=-1)
    return jnp.einsum("bhqk,bhkd->bhqd", p, v)
```

```python
import math

import jax
import jax.numpy as jnp
from jax import lax
import jax.experimental.pallas as pl
import jax.experimental.pallas.tpu as pltpu

WINDOW = 32
KT = 128
QT = KT - WINDOW
MASKED = -1e30

READ_SLOTS = 2
GROUPS = 8
WROWS = 64


def _attend(q, k, v, bias, c):
    s = lax.dot_general(q, k, (((1,), (1,)), ((), ())), preferred_element_type=jnp.float32)
    s = s + bias
    m = jnp.max(s, axis=-1, keepdims=True)
    p = jnp.exp2((s - m) * c)
    l = jnp.sum(p, axis=-1, keepdims=True)
    o = jnp.dot(p.astype(v.dtype), v, preferred_element_type=jnp.float32)
    return o * (1.0 / l)


def _kernel(q_hbm, k_hbm, v_hbm, o_hbm, qb, kb, vb, ob, sem):
    H, S, D = q_hbm.shape
    G, HG = o_hbm.shape[:2]
    c = (D ** -0.5) * math.log2(math.e)
    srcs = (q_hbm, k_hbm, v_hbm)
    bufs = (qb, kb, vb)

    def read(a, h, slot):
        return pltpu.make_async_copy(srcs[a].at[h], bufs[a].at[h], sem.at[slot])

    wslot = (H - 2) % READ_SLOTS
    wblocks = [(j, s) for j in range(HG) for s in range(S // WROWS)]
    n_early = (HG - 1) * (S // WROWS)

    def write(i):
        j, s = wblocks[i]
        sl = (slice(None), j, pl.ds(s * WROWS, WROWS))
        return pltpu.make_async_copy(ob.at[sl], o_hbm.at[sl], sem.at[wslot])

    def compute(h):
        g = h // HG
        j = h % HG
        rel = (lax.broadcasted_iota(jnp.int32, (KT, KT), 0)
               - lax.broadcasted_iota(jnp.int32, (KT, KT), 1))
        bias = jnp.where((rel >= 0) & (rel < WINDOW), 0.0, MASKED).astype(jnp.float32)
        ob[g, j, 0:KT, :] = _attend(
            qb[h, 0:KT, :], kb[h, 0:KT, :], vb[h, 0:KT, :], bias, c).astype(ob.dtype)
        tail = bias[WINDOW:, :]
        for t in range(1, (S - KT) // QT + 1):
            ks = QT * t
            qs = ks + WINDOW
            ob[g, j, qs:qs + QT, :] = _attend(
                qb[h, qs:qs + QT, :], kb[h, ks:ks + KT, :], vb[h, ks:ks + KT, :],
                tail, c).astype(ob.dtype)

    for h in range(READ_SLOTS):
        for a in range(3):
            read(a, h, h).start()

    def body(h, carry):
        slot = lax.rem(h, READ_SLOTS)
        for a in range(3):
            read(a, h, slot).wait()

        @pl.when(h + READ_SLOTS < H)
        def _():
            for a in range(3):
                read(a, h + READ_SLOTS, slot).start()

        compute(h)
        return carry

    lax.fori_loop(0, H - 1, body, 0)

    last = H - 1
    read(0, last, last % READ_SLOTS).wait()
    read(1, last, last % READ_SLOTS).wait()
    for i in range(n_early):
        write(i).start()
    read(2, last, last % READ_SLOTS).wait()
    compute(last)
    for i in range(n_early, len(wblocks)):
        write(i).start()
    for i in range(len(wblocks)):
        write(i).wait()


@jax.jit
def pallas_standalone__sliding_local_fixed_window__prompt_kernel(
    q: jax.Array,
    k: jax.Array,
    v: jax.Array,
):
    B, H, S, D = q.shape
    BH = B * H
    assert D == KT and (S - KT) % QT == 0 and S % WROWS == 0
    assert BH % GROUPS == 0 and BH > READ_SLOTS
    in_shape = (BH, S, D)
    out_shape = (GROUPS, BH // GROUPS, S, D)
    any_spec = pl.BlockSpec(memory_space=pl.ANY)
    out = pl.pallas_call(
        _kernel,
        in_specs=[any_spec, any_spec, any_spec],
        out_specs=any_spec,
        out_shape=jax.ShapeDtypeStruct(out_shape, q.dtype),
        scratch_shapes=[
            pltpu.VMEM(in_shape, q.dtype),
            pltpu.VMEM(in_shape, k.dtype),
            pltpu.VMEM(in_shape, v.dtype),
            pltpu.VMEM(out_shape, q.dtype),
            pltpu.SemaphoreType.DMA((READ_SLOTS,)),
        ],
        compiler_params=pltpu.CompilerParams(vmem_limit_bytes=100 * 1024 * 1024),
    )(q.reshape(in_shape), k.reshape(in_shape), v.reshape(in_shape))
    return out.reshape(q.shape)
```

```python
import math

import jax
import jax.numpy as jnp
from jax import lax
import jax.experimental.pallas as pl
import jax.experimental.pallas.tpu as pltpu

WINDOW = 32
KT = 128
QT = KT - WINDOW
MASKED = -1e30

RHEADS = 4
RROWS = 16
LOOKAHEAD = 6
TAIL_ROWS = 448
WPIECES = 8
WROWS = 64


def _attend(q, k, v, mask, c):
    s = lax.dot_general(q, k, (((1,), (1,)), ((), ())), preferred_element_type=jnp.float32)
    s = jnp.where(mask, s, MASKED)
    m = jnp.max(s, axis=-1, keepdims=True)
    p = jnp.exp2((s - m) * c)
    l = jnp.sum(p, axis=-1, keepdims=True)
    o = jnp.dot(p.astype(v.dtype), v, preferred_element_type=jnp.float32)
    return o * (1.0 / l)


def _kernel(q_hbm, k_hbm, v_hbm, o_hbm, qb, kb, vb, ob, sem):
    _, NG, S, D = q_hbm.shape
    HW = o_hbm.shape[1]
    H = RHEADS * NG
    step_rows = S // RHEADS
    n_tiles = (S - KT) // QT + 1
    c = (D ** -0.5) * math.log2(math.e)
    srcs = (q_hbm, k_hbm, v_hbm)
    bufs = (qb, kb, vb)

    chunks = [(i, a) for i in range(step_rows // RROWS) for a in range(3)]

    def start_reads(step, lo, hi):
        g = step // RHEADS
        r0 = (step % RHEADS) * step_rows
        for i, a in chunks[lo:hi]:
            off = r0 + i * RROWS
            if not isinstance(off, int):
                off = pl.multiple_of(off, RROWS)
            sl = (slice(None), g, pl.ds(off, RROWS))
            pltpu.make_async_copy(srcs[a].at[sl], bufs[a].at[sl], sem.at[g % 2]).start(
                priority=0 if a == 2 else 1)

    def wait_reads(a, g, lo, hi):
        sl = (slice(None), g, pl.ds(lo, hi - lo))
        pltpu.make_async_copy(srcs[a].at[sl], bufs[a].at[sl], sem.at[g % 2]).wait()

    wblocks = [(j, s) for j in range(HW) for s in range(S // WROWS)]

    def write(i):
        j, s = wblocks[i]
        sl = (slice(None), j, pl.ds(s * WROWS, WROWS))
        return pltpu.make_async_copy(ob.at[sl], o_hbm.at[sl], sem.at[(NG - 2) % 2])

    def compute(hh, step):
        g = hh // RHEADS
        n = hh % RHEADS
        head = NG * n + g
        gw = head // HW
        j = head % HW
        rel = (lax.broadcasted_iota(jnp.int32, (KT, KT), 0)
               - lax.broadcasted_iota(jnp.int32, (KT, KT), 1))
        mask = (rel >= 0) & (rel < WINDOW)
        for t in range(n_tiles):
            if step is not None:
                start_reads(step, len(chunks) * t // n_tiles, len(chunks) * (t + 1) // n_tiles)
            ks = QT * t
            skip = 0 if t == 0 else WINDOW
            qs = ks + skip
            ob[gw, j, qs:ks + KT, :] = _attend(
                qb[n, g, qs:ks + KT, :], kb[n, g, ks:ks + KT, :], vb[n, g, ks:ks + KT, :],
                mask[skip:, :], c).astype(ob.dtype)

    for step in range(LOOKAHEAD):
        start_reads(step, 0, len(chunks))

    def read_body(hh, carry):
        @pl.when(hh % RHEADS == 0)
        def _():
            for a in range(3):
                wait_reads(a, hh // RHEADS, 0, S)

        compute(hh, hh + LOOKAHEAD)
        return carry

    lax.fori_loop(0, H - LOOKAHEAD, read_body, 0)

    last = NG - 1
    wait_reads(0, last, 0, S)
    wait_reads(1, last, 0, S)
    wait_reads(2, last, 0, S - TAIL_ROWS)
    n_first = len(wblocks) // 2
    for i in range(n_first):
        write(i).start()

    def tail_body(hh, carry):
        @pl.when(hh == H - RHEADS)
        def _():
            wait_reads(2, last, S - TAIL_ROWS, S)

        compute(hh, None)
        return carry

    lax.fori_loop(H - LOOKAHEAD, H, tail_body, 0)
    for i in range(n_first, len(wblocks)):
        write(i).start()
    for i in range(len(wblocks)):
        write(i).wait()


@jax.jit
def pallas_standalone__sliding_local_fixed_window__prompt_kernel(
    q: jax.Array,
    k: jax.Array,
    v: jax.Array,
):
    B, H, S, D = q.shape
    BH = B * H
    NG = BH // RHEADS
    HW = BH // WPIECES
    assert D == KT and (S - KT) % QT == 0 and S % (RHEADS * RROWS) == 0 and S % WROWS == 0
    assert BH % RHEADS == 0 and BH % WPIECES == 0 and RHEADS <= LOOKAHEAD < 2 * RHEADS
    assert NG % HW == 0 and HW % 2 == 0 and NG - HW + HW // 2 <= NG - 2
    in_shape = (RHEADS, NG, S, D)
    out_shape = (WPIECES, HW, S, D)
    any_spec = pl.BlockSpec(memory_space=pl.ANY)
    out = pl.pallas_call(
        _kernel,
        in_specs=[any_spec, any_spec, any_spec],
        out_specs=any_spec,
        out_shape=jax.ShapeDtypeStruct(out_shape, q.dtype),
        scratch_shapes=[
            pltpu.VMEM(in_shape, q.dtype),
            pltpu.VMEM(in_shape, k.dtype),
            pltpu.VMEM(in_shape, v.dtype),
            pltpu.VMEM(out_shape, q.dtype),
            pltpu.SemaphoreType.DMA((2,)),
        ],
        compiler_params=pltpu.CompilerParams(
            vmem_limit_bytes=100 * 1024 * 1024,
            disable_bounds_checks=True,
        ),
    )(q.reshape(in_shape), k.reshape(in_shape), v.reshape(in_shape))
    return out.reshape(q.shape)
```
